```python
import os as _os
_os.environ.setdefault("JAX_PLATFORMS", "cpu")
import jax
import jax.numpy as jnp

def _softmax(x, axis=-1):
    return jax.nn.softmax(x, axis=axis)
def _gelu(x):
    return jax.nn.gelu(x, approximate=True)
def _silu(x):
    return jax.nn.silu(x)
def _sigmoid(x):
    return jax.nn.sigmoid(x)
def _layernorm(x, axis=-1, eps=1e-5):
    m = jnp.mean(x, axis=axis, keepdims=True)
    v = jnp.var(x, axis=axis, keepdims=True)
    return (x - m) / jnp.sqrt(v + eps)
def _scatter_add(tgt, idx, src, axis=0):
    return tgt.at[idx].add(src)
def _segment_sum(src, seg, n):
    return jax.ops.segment_sum(src, seg, n)
class _Rng:
    def __init__(self, key):
        self._k = key
    def _next(self):
        self._k, sub = jax.random.split(self._k)
        return sub
    def normal(self, shape):
        return jax.random.normal(self._next(), shape, dtype=jnp.bfloat16)
    def randint(self, lo, hi, shape):
        return jax.random.randint(self._next(), shape, lo, hi, dtype=jnp.int32)
    def uniform(self, shape, lo=0.0, hi=1.0):
        return jax.random.uniform(self._next(), shape, jnp.bfloat16, lo, hi)
    def permutation(self, n):
        return jax.random.permutation(self._next(), n)


kernel_name = 'gated_mix__linear_attn_block__sliding_local_dilated__prompt'

def setup_inputs():
    _rng = _Rng(jax.random.key(int.from_bytes(__import__("os").urandom(4), "little")))
    _w = (lambda a: (lambda t: t.astype(jnp.bfloat16) if jnp.issubdtype(t.dtype, jnp.floating) else t)(jnp.asarray(a)))
    def _A_setup():
        B, S, D = 1, 2048, 512
        return {
            "x": _w((lambda *s: _rng.normal(s) * 0.05)(B, S, D)),
            "wqkv": _w((lambda *s: _rng.normal(s) * 1.6)(D, 3 * D)),
            "wo": _w((lambda *s: _rng.normal(s) * 0.8)(D, D)),
        }
    _A_in = _A_setup()

    def _B_setup():
        B, S, D = 1, 2048, 512
        return {
            "x": _w((lambda *s: _rng.normal(s) * 0.05)(B, S, D)),
            "wqkv": _w((lambda *s: _rng.normal(s) * 0.8)(D, 3 * D)),
            "wo": _w((lambda *s: _rng.normal(s) * 0.05)(D, D)),
        }
    _B_in = _B_setup()

    return {
        "A_x": _A_in["x"],
        "A_wqkv": _A_in["wqkv"],
        "A_wo": _A_in["wo"],
        "B_x": _B_in["x"],
        "B_wqkv": _B_in["wqkv"],
        "B_wo": _B_in["wo"],
        "gate_w": _w((lambda *s: _rng.normal(s) * 0.05)(512) * 16.0),
    }

def reference(A_x, A_wqkv, A_wo, B_x, B_wqkv, B_wo, gate_w):
    def _A_ref(x, wqkv, wo):
        B, S, D = x.shape
        H = 32; Dh = D // H
        qkv = (lambda x, *d: x.transpose(*d))((x @ wqkv).reshape(B, S, 3, H, Dh), 2, 0, 3, 1, 4)
        q, k, v = qkv[0], qkv[1], qkv[2]
        phi = lambda t: jnp.where(t > 0, t + 1, jnp.exp(t)) + 1e-6
        pq, pk = phi(q), phi(k)
        kv = jnp.einsum("bhsd,bhse->bhde", pk, v)
        z = jnp.einsum("bhsd->bhd", pk)
        num = jnp.einsum("bhqd,bhde->bhqe", pq, kv)
        den = jnp.einsum("bhqd,bhd->bhq", pq, z)[..., None] + 1e-6
        o = num / den
        return (lambda x, *d: x.transpose(*d))(o, 0, 2, 1, 3).reshape(B, S, D) @ wo

    def _B_ref(x, wqkv, wo):
        B, S, D = x.shape
        H = 32; Dh = D // H
        W, dil = 8, 2
        qkv = (lambda x, *d: x.transpose(*d))((x @ wqkv).reshape(B, S, 3, H, Dh), 2, 0, 3, 1, 4)
        q, k, v = qkv[0], qkv[1], qkv[2]
        scale = Dh ** -0.5
        pos = jnp.arange(S)
        off = jnp.arange(W) * dil
        idx = pos[:, None] - off[None, :]
        mask = idx >= 0
        idx_c = jnp.where(mask, idx, 0).reshape(-1)
        kg = k[:, :, idx_c, :].reshape(B, H, S, W, Dh)
        vg = v[:, :, idx_c, :].reshape(B, H, S, W, Dh)
        logits = jnp.einsum("bhsd,bhswd->bhsw", q, kg) * scale
        logits = jnp.where(mask[None, None, :, :], logits, -1e9)
        attn = _softmax(logits, axis=-1)
        o = jnp.einsum("bhsw,bhswd->bhsd", attn, vg)
        return (lambda x, *d: x.transpose(*d))(o, 0, 2, 1, 3).reshape(B, S, D) @ wo

    x = A_x
    g = _sigmoid((x * gate_w).sum(-1, keepdims=True))
    a = _A_ref(x, A_wqkv, A_wo)
    b = _B_ref(x, B_wqkv, B_wo)
    return g * a + (1 - g) * b
```

```python
import numpy as np
import jax
import jax.numpy as jnp
import jax.experimental.pallas as pl
import jax.experimental.pallas.tpu as pltpu

S, D, H, DH, W, DIL = 2048, 512, 32, 16, 8, 2
T1 = 512
T = 256
ORDER = 1
HALO = 16
TT = T + HALO
PI = 2
DM = 0
CH = 32
FS = 0
F32, BF16, U32 = jnp.float32, jnp.bfloat16, jnp.uint32
LOG2E = 1.4426950408889634


def _phi(t):
    return jnp.where(t > 0, t + 1.0, jnp.exp(t)) + 1e-6


def _pk(x):
    return pltpu.bitcast(x, U32)


def _upk(x):
    return pltpu.bitcast(x, BF16)


def _perm_cols(w):
    R = w.shape[0]
    lane = jax.lax.broadcasted_iota(jnp.int32, (R, 128), 1)
    j_of = (lane % 32) // 8
    outs = []
    for g in range(4):
        idx = (lane % 8) * 16 + 4 * g + lane // 32
        acc = None
        for j in range(4):
            t = jnp.take_along_axis(w[:, 128 * j:128 * (j + 1)], idx, axis=1)
            acc = t if acc is None else jnp.where(j_of == j, t, acc)
        outs.append(acc)
    return outs


def _kernel(xa_hbm, wa_hbm, woa_hbm, wb_hbm, wob_hbm, gw_ref, out_hbm,
            xa, wa, woa, wb, wob, xp, wf, wkt, pacc, zacc, mw, tmp, qs, ks, vs, lh, ob, sems, osems):
    NX = S // T1
    cps = [pltpu.make_async_copy(wa_hbm.at[:, D:2 * D], wa.at[:, D:2 * D], sems.at[0])]
    for i in range(NX):
        cps.append(pltpu.make_async_copy(xa_hbm.at[i * T1:(i + 1) * T1], xa.at[i * T1:(i + 1) * T1], sems.at[1 + i]))
    c_wq = pltpu.make_async_copy(wa_hbm.at[:, 0:D], wa.at[:, 0:D], sems.at[NX + 1])
    c_wv = pltpu.make_async_copy(wa_hbm.at[:, 2 * D:], wa.at[:, 2 * D:], sems.at[NX + 2])
    c_wb = pltpu.make_async_copy(wb_hbm, wb, sems.at[NX + 3])
    c_woa = pltpu.make_async_copy(woa_hbm, woa, sems.at[NX + 4])
    c_wob = pltpu.make_async_copy(wob_hbm, wob, sems.at[NX + 5])
    cps[0].start(); cps[1].start()
    cps[0].wait()
    cps[2].start()
    if DM == 0:
        cps[3].start(); c_wq.start()
    wkt[...] = _pk(wa[:, D:2 * D].astype(F32).T.astype(BF16))
    cps[1].wait()
    if DM == 1:
        cps[3].start(); c_wq.start()
    c_wb.start(); cps[4].start(); c_wob.start(); c_wv.start(); c_woa.start()

    def p1(i, first):
        r0 = pl.multiple_of(i * T1, T1)
        xt = xa[pl.ds(r0, T1), :]
        xp[pl.ds(pl.multiple_of(i * (T1 // 2), T1 // 2), T1 // 2), :] = _pk(xt)
        kt = jax.lax.dot_general(_upk(wkt[...]), xt, (((1,), (1,)), ((), ())), preferred_element_type=F32)
        pk = _phi(kt)
        zp = pk[:, 0:128]
        for j in range(1, T1 // 128):
            zp = zp + pk[:, 128 * j:128 * (j + 1)]
        pp = jnp.dot(pk.astype(BF16), xt, preferred_element_type=F32)
        zacc[...] += zp
        pacc[...] += pp
        if first:
            return
        RW = D // (NX - PI)
        w0 = pl.multiple_of((i - PI) * RW, RW)
        p0 = pl.multiple_of((i - PI) * (RW // 2), RW // 2)
        for c in range(4):
            src = wa[pl.ds(w0, RW), 0:D] if c == 0 else wb[pl.ds(w0, RW), (c - 1) * D:c * D]
            o = _perm_cols(_pk(src))
            for g in range(4):
                wf[pl.ds(p0, RW // 2), c * D + 128 * g:c * D + 128 * (g + 1)] = o[g]

    pacc[...] = jnp.zeros_like(pacc)
    zacc[...] = jnp.zeros_like(zacc)
    cps[2].wait()
    def pa(i, _):
        p1(i, True)
        return 0
    jax.lax.fori_loop(0, 2, pa, 0)
    cps[3].wait(); cps[4].wait(); c_wob.wait(); c_wv.wait(); c_woa.wait(); c_wq.wait(); c_wb.wait()
    def pb(i, _):
        p1(i, False)
        return 0
    jax.lax.fori_loop(2, 4, pb, 0)
    for g in range(4):
        tmp[g] = wob[:, 128 * g:128 * (g + 1)].astype(F32)
    for g in range(4):
        for d in range(DH):
            mw[D // 2 + d * 16:D // 2 + (d + 1) * 16, 128 * g:128 * (g + 1)] = _pk(tmp[g, pl.ds(d, H, stride=DH), :].astype(BF16))
    row = jax.lax.broadcasted_iota(jnp.int32, (128, 128), 0)
    col = jax.lax.broadcasted_iota(jnp.int32, (128, 128), 1)
    same = (row // DH) == (col // DH)
    for j in range(4):
        p = pacc[128 * j:128 * (j + 1), :]
        ph = p.astype(BF16)
        plo = (p - ph.astype(F32)).astype(BF16)
        wv = wa[:, 2 * D + 128 * j:2 * D + 128 * (j + 1)]
        kv = jnp.dot(ph, wv, preferred_element_type=F32) + jnp.dot(plo, wv, preferred_element_type=F32)
        kv = jnp.where(same, kv, 0.0).astype(BF16)
        mj = jnp.dot(kv, woa[128 * j:128 * (j + 1), :], preferred_element_type=F32)
        for g in range(4):
            tmp[g, 128 * j:128 * (j + 1), :] = mj[:, 128 * g:128 * (g + 1)]
    for g in range(4):
        for d in range(DH):
            mw[d * 16:(d + 1) * 16, 128 * g:128 * (g + 1)] = _pk(tmp[g, pl.ds(d, H, stride=DH), :].astype(BF16))
    zr = []
    for g in range(4):
        zp = jnp.concatenate([zacc[pl.ds(4 * g + dl, H, stride=DH), :] for dl in range(4)], axis=0)
        zr.append(jnp.sum(zp.T, axis=0, keepdims=True))
    for g in range(4):
        ks[g, TT + T:2 * TT, :] = jnp.zeros((HALO, 128), F32)
        vs[g, TT + T:2 * TT, :] = jnp.zeros((HALO, 128), F32)
    gw = gw_ref[...].astype(F32).reshape(1, D)

    def proj(i, sl):
        r0 = sl * TT
        xt = _upk(xp[pl.ds(pl.multiple_of(i * (T // 2), T // 2), T // 2), :])
        ro = (1 - sl) * TT
        for g in range(4):
            ks[g, r0:r0 + HALO, :] = ks[g, ro + T:ro + TT, :]
            vs[g, r0:r0 + HALO, :] = vs[g, ro + T:ro + TT, :]
        g_ = jax.nn.sigmoid(jnp.sum(xt.astype(F32) * gw, axis=1, keepdims=True))
        g_ = jnp.broadcast_to(g_, (T, 128))
        pq = [_phi(jnp.dot(xt, _upk(wf[:, 128 * g:128 * (g + 1)]), preferred_element_type=F32)) for g in range(4)]
        den = pq[0] * zr[0]
        for g in range(1, 4):
            den = den + pq[g] * zr[g]
        den = den + pltpu.roll(den, 64, 1)
        den = den + pltpu.roll(den, 32, 1)
        r = g_ / (den + 1e-6)
        for g in range(4):
            lh[sl * T // 2:(sl + 1) * T // 2, 128 * g:128 * (g + 1)] = _pk((pq[g] * r).astype(BF16))
        qs[4, r0:r0 + T, :] = 1.0 - g_
        for c, dst, off in ((1, qs, 0), (2, ks, HALO), (3, vs, HALO)):
            for g in range(4):
                y = jnp.dot(xt, _upk(wf[:, c * D + 128 * g:c * D + 128 * (g + 1)]), preferred_element_type=F32)
                if c == 1:
                    y = y * (0.25 * LOG2E)
                dst[g, off + r0:off + r0 + T, :] = y

    def attn(i, sl, r_lo, n):
        r0 = sl * TT + r_lo
        l0 = sl * T + r_lo
        ls = []
        for w in range(W):
            o = HALO + r0 - DIL * w
            l = qs[0, r0:r0 + n, :] * ks[0, o:o + n, :]
            for g in range(1, 4):
                l = l + qs[g, r0:r0 + n, :] * ks[g, o:o + n, :]
            l = l + pltpu.roll(l, 64, 1)
            l = l + pltpu.roll(l, 32, 1)
            if w > 0 and r_lo < DIL * w:
                pos = i * T + r_lo + jax.lax.broadcasted_iota(jnp.int32, (n, 128), 0)
                l = jnp.where(pos >= DIL * w, l, -1e9)
            ls.append(l)
        m = ls[0]
        for w in range(1, W):
            m = jnp.maximum(m, ls[w])
        es = [jnp.exp2(l - m) for l in ls]
        ssum = es[0]
        for w in range(1, W):
            ssum = ssum + es[w]
        r = qs[4, r0:r0 + n, :] / ssum
        for g in range(4):
            acc = es[0] * vs[g, HALO + r0:HALO + r0 + n, :]
            for w in range(1, W):
                o = HALO + r0 - DIL * w
                acc = acc + es[w] * vs[g, o:o + n, :]
            lh[l0 // 2:(l0 + n) // 2, D + 128 * g:D + 128 * (g + 1)] = _pk((acc * r).astype(BF16))

    def attn_tile(i, sl):
        for r in range(0, T, CH):
            attn(i, sl, r, CH)

    NT = S // T
    def ocp(i):
        return pltpu.make_async_copy(ob.at[pl.ds(pl.multiple_of(i * T, T), T), :], out_hbm.at[pl.ds(pl.multiple_of(i * T, T), T), :], osems.at[i])
    def final(i, sl):
        l = _upk(lh[sl * T // 2:(sl + 1) * T // 2, :])
        for g in range(4):
            ob[pl.ds(pl.multiple_of(i * T, T), T), 128 * g:128 * (g + 1)] = jnp.dot(l, _upk(mw[:, 128 * g:128 * (g + 1)]), preferred_element_type=F32).astype(BF16)
    proj(0, 0)
    def body(j, _):
        i = 2 * j
        proj(i + 1, 1); attn_tile(i, 0)
        if ORDER == 1:
            final(i, 0)
        proj(i + 2, 0); attn_tile(i + 1, 1)
        if ORDER != 1:
            final(i, 0)
        final(i + 1, 1)
        ocp(i).start(); ocp(i + 1).start()
        return 0
    jax.lax.fori_loop(0, NT // 2 - 1, body, 0)
    proj(NT - 1, 1); attn_tile(NT - 2, 0); final(NT - 2, 0); ocp(NT - 2).start()
    attn_tile(NT - 1, 1); final(NT - 1, 1); ocp(NT - 1).start()
    for i in range(NT):
        ocp(i).wait()


@jax.jit
def pallas_gated_mix__linear_attn_block__sliding_local_dilated__prompt_kernel(A_x, A_wqkv, A_wo, B_x, B_wqkv, B_wo, gate_w):
    anyspec = pl.BlockSpec(memory_space=pl.ANY)
    out = pl.pallas_call(
        _kernel,
        out_shape=jax.ShapeDtypeStruct((S, D), BF16),
        in_specs=[anyspec] * 5 + [pl.BlockSpec(memory_space=pltpu.VMEM)],
        out_specs=anyspec,
        scratch_shapes=[
            pltpu.VMEM((S, D), BF16),
            pltpu.VMEM((D, 3 * D), BF16), pltpu.VMEM((D, D), BF16),
            pltpu.VMEM((D, 3 * D), BF16), pltpu.VMEM((D, D), BF16),
            pltpu.VMEM((S // 2, D), U32), pltpu.VMEM((D // 2, 4 * D), U32), pltpu.VMEM((D // 2, D), U32),
            pltpu.VMEM((D, D), F32), pltpu.VMEM((D, 128), F32),
            pltpu.VMEM((D, D), U32), pltpu.VMEM((4, D, 128), F32),
            pltpu.VMEM((5, 2 * TT, 128), F32),
            pltpu.VMEM((4, 2 * TT, 128), F32), pltpu.VMEM((4, 2 * TT, 128), F32),
            pltpu.VMEM((T, 2 * D), U32),
            pltpu.VMEM((S, D), BF16),
            pltpu.SemaphoreType.DMA((S // T1 + 6,)), pltpu.SemaphoreType.DMA((S // T,)),
        ],
        compiler_params=pltpu.CompilerParams(vmem_limit_bytes=100 * 1024 * 1024),
    )(A_x.reshape(S, D), A_wqkv, A_wo, B_wqkv, B_wo, gate_w)
    return out.reshape(1, S, D)
```
